```python
import jax
import jax.numpy as jnp

def _softmax(x, axis=-1):
    return jax.nn.softmax(x, axis=axis)
def _gelu(x):
    return jax.nn.gelu(x, approximate=True)
def _silu(x):
    return jax.nn.silu(x)
def _sigmoid(x):
    return jax.nn.sigmoid(x)
def _layernorm(x, axis=-1, eps=1e-5):
    m = jnp.mean(x, axis=axis, keepdims=True)
    v = jnp.var(x, axis=axis, keepdims=True)
    return (x - m) / jnp.sqrt(v + eps)
def _scatter_add(tgt, idx, src, axis=0):
    return tgt.at[idx].add(src)
def _segment_sum(src, seg, n):
    return jax.ops.segment_sum(src, seg, n)
class _Rng:
    def __init__(self, key):
        self._k = key
    def _next(self):
        self._k, sub = jax.random.split(self._k)
        return sub
    def normal(self, shape):
        return jax.random.normal(self._next(), shape, dtype=jnp.bfloat16)
    def randint(self, lo, hi, shape):
        return jax.random.randint(self._next(), shape, lo, hi, dtype=jnp.int32)
    def uniform(self, shape, lo=0.0, hi=1.0):
        return jax.random.uniform(self._next(), shape, jnp.bfloat16, lo, hi)
    def permutation(self, n):
        return jax.random.permutation(self._next(), n)


kernel_name = 'standalone__seq2seq_rnn_t_joint__speech'

def _fwd_setup_inputs():
    _rng = _Rng(jax.random.key(int.from_bytes(__import__("os").urandom(4), "little")))
    _w = (lambda a: (lambda t: t.astype(jnp.bfloat16) if jnp.issubdtype(t.dtype, jnp.floating) else t)(jnp.asarray(a)))
    B, T, D, K = 2, 4000, 256, 3
    U = 8
    sc = (1.0 / (K * D)) ** 0.5
    sd = (1.0 / D) ** 0.5
    return {
        "x": _w((lambda *s: _rng.normal(s) * 0.05)(B, T, D) * 0.5),
        "w1": _w((lambda *s: _rng.normal(s) * 0.05)(K, D, D) * sc),
        "w2": _w((lambda *s: _rng.normal(s) * 0.05)(K, D, D) * sc),
        "g": _w((lambda *s: _rng.normal(s) * 0.05)(B, U, D) * 0.5),
        "w_f": _w((lambda *s: _rng.normal(s) * 0.05)(D, D) * sd),
        "w_g": _w((lambda *s: _rng.normal(s) * 0.05)(D, D) * sd),
        "w_o": _w((lambda *s: _rng.normal(s) * 0.05)(D, D) * sd),
    }

def _fwd_reference(x, w1, w2, g, w_f, w_g, w_o):
    B, T, D = x.shape
    K = w1.shape[0]
    pad = K // 2
    xp = jnp.pad(x, ((0,0),(pad,pad),(0,0)))
    h = jnp.zeros_like(x)
    for i in range(K):
        h = h + jnp.einsum("btc,cd->btd", xp[:, i:i+T, :], w1[i])
    h = _gelu(h)[:, ::2, :]
    T1 = h.shape[1]
    hp = jnp.pad(h, ((0,0),(pad,pad),(0,0)))
    f = jnp.zeros_like(h)
    for i in range(K):
        f = f + jnp.einsum("btc,cd->btd", hp[:, i:i+T1, :], w2[i])
    f = _gelu(f)[:, ::2, :]
    fe = jnp.einsum("btd,de->bte", f, w_f)
    ge = jnp.einsum("bud,de->bue", g, w_g)
    j = jnp.tanh(fe[:, :, None, :] + ge[:, None, :, :])
    return jnp.einsum("btud,dv->btuv", j, w_o)


def setup_inputs():
    _inp = _fwd_setup_inputs()
    _gk = jax.random.fold_in(jax.random.key(int.from_bytes(__import__("os").urandom(4), "little")), 2**31 - 1)
    _shapes = [[2, 1000, 8, 256]]
    _dtypes = ['bfloat16']
    _gks = jax.random.split(_gk, len(_shapes))
    _gs = [jax.random.normal(k, s, dtype=jnp.dtype(d)) * 0.05 for k, s, d in zip(_gks, _shapes, _dtypes)]
    _inp["grad_out"] = _gs[0]
    return _inp

def reference(x, w1, w2, g, w_f, w_g, w_o, grad_out):
    _const = dict()
    def _f(*_d):
        return _fwd_reference(**{'x': _d[0], 'w1': _d[1], 'w2': _d[2], 'g': _d[3], 'w_f': _d[4], 'w_g': _d[5], 'w_o': _d[6], **_const})
    _out, _vjp = jax.vjp(_f, x, w1, w2, g, w_f, w_g, w_o)
    _grads = _vjp(grad_out)
    _out0 = jnp.asarray(_out)
    return (_out0, *[jnp.asarray(_g) for _g in _grads])
```

```python
import jax
import jax.numpy as jnp
from jax import lax
from jax.experimental import pallas as pl
from jax.experimental.pallas import tpu as pltpu

f32 = jnp.float32
bf16 = jnp.bfloat16
u32 = jnp.uint32

B, T, D, U = 2, 4000, 256, 8
R = 1000
TR = 250
NT = R // TR
NSTEP = B * NT
M = 256
Q = M // 2
H = 128
XW = 1040
XD = 1016
GW = M * U + 8
GD = (TR + 1) * U
DXW = 1040

GELU_C0 = 0.7978845608028654
GELU_C1 = 0.044715


def _nn(a, w):
    return jnp.dot(a, w, preferred_element_type=f32)


def _nt(a, w):
    return lax.dot_general(a, w, (((1,), (1,)), ((), ())), preferred_element_type=f32)


def _tn(a, b):
    return lax.dot_general(a, b, (((0,), (0,)), ((), ())), preferred_element_type=f32)


def _gelu_and_grad(x):
    x2 = x * x
    th = jnp.tanh(x * (GELU_C0 + (GELU_C0 * GELU_C1) * x2))
    s = 0.5 + 0.5 * th
    g = x * s
    dg = s + x * (1.0 - th * th) * (0.5 * GELU_C0 + (1.5 * GELU_C0 * GELU_C1) * x2)
    return g, dg


def _cat(lo, hi):
    return jnp.concatenate([lo, hi], axis=1)


def _stack(a, b):
    return jnp.concatenate([a, b], axis=0)


def _halves(v):
    return v[:, :H], v[:, H:]


def _keep_rows(v, lo, hi):
    n = v.shape[0]
    a = -(-lo // 8) * 8
    b = hi // 8 * 8
    zero = jnp.zeros((), v.dtype)
    parts = []
    if a > 0:
        r = lax.broadcasted_iota(jnp.int32, (a, v.shape[1]), 0)
        parts.append(jnp.where(r >= lo, v[:a], zero))
    parts.append(v[a:b])
    if b < n:
        r = lax.broadcasted_iota(jnp.int32, (n - b, v.shape[1]), 0) + b
        parts.append(jnp.where(r < hi, v[b:], zero))
    return jnp.concatenate(parts, axis=0)


def _keep_even(v):
    return _keep_rows(v, 1, TR // 2 + 1)


def _keep_odd(v):
    return _keep_rows(v, 0, TR // 2)


def _keep_valid(v):
    return _stack(_keep_even(v[:Q]), _keep_odd(v[Q:]))


def _zero_row_if(v, row, cond):
    if cond is False:
        return v
    a = row // 8 * 8
    blk = v[a:a + 8]
    r = lax.broadcasted_iota(jnp.int32, blk.shape, 0) + a
    kill = row if cond is True else jnp.where(cond, row, -1)
    blk = jnp.where(r == kill, jnp.zeros((), v.dtype), blk)
    parts = ([v[:a]] if a > 0 else []) + [blk] + ([v[a + 8:]] if a + 8 < v.shape[0] else [])
    return jnp.concatenate(parts, axis=0)


def _lo(w):
    return pltpu.unpack_elementwise(w, index=0, packed_dtype=bf16, unpacked_dtype=f32)


def _hi(w):
    return pltpu.unpack_elementwise(w, index=1, packed_dtype=bf16, unpacked_dtype=f32)


def _pack(a, b):
    return pltpu.pack_elementwise([a, b], packed_dtype=bf16)


def _words(v):
    return pltpu.bitcast(v, u32)


def _rows(w):
    return pltpu.bitcast(w, bf16)


def _aligned(v):
    return v if isinstance(v, int) else pl.multiple_of(v, 8)


def _kernel(x_hbm, go_hbm, g_hbm, w1_hbm, w2_hbm, wf_hbm, wg_hbm, wo_hbm,
            out_hbm, dx_hbm, dw1_hbm, dw2_hbm, dg_hbm, dwf_hbm, dwg_hbm, dwo_hbm,
            xbuf, gbuf, obuf, dxbuf,
            g_ref, w1_ref, w2_ref, wf_ref, wg_ref, wo_ref, ws_ref, vs_ref,
            at_ref, het_ref, ht_ref, f_ref, ghe_ref, gho_ref, gf_ref, fe_ref, j_ref, jt_ref,
            shift_a, shift_b, shift_c, fold, ge_ref,
            acc1, acc2, accf, acco, accg, dge_ref,
            dw1_st, dw2_st, dwf_st, dwo_st, dwg_st, dg_st,
            in_sem, out_sem, w_sem, dw_sem):

    def x_copy(step, h):
        nominal = step * (4 * TR) - 8
        if isinstance(step, int):
            src = min(max(nominal, 0), B * T - XD)
        else:
            src = jnp.clip(nominal, 0, B * T - XD)
        return pltpu.make_async_copy(
            x_hbm.at[pl.ds(_aligned(src), XD), pl.ds(h * H, H)],
            xbuf.at[step, h, pl.ds(_aligned(8 + src - nominal), XD), :],
            in_sem.at[step, h])

    def g_copy(step, h):
        nominal = step * TR
        if isinstance(step, int):
            src = min(nominal, B * R - (TR + 1))
        else:
            src = jnp.minimum(nominal, B * R - (TR + 1))
        return pltpu.make_async_copy(
            go_hbm.at[pl.ds(_aligned(src * U), GD), pl.ds(h * H, H)],
            gbuf.at[step, h, pl.ds(_aligned((1 + src - nominal) * U), GD), :],
            in_sem.at[step, 2 + h])

    def o_copy(step, h):
        return pltpu.make_async_copy(
            obuf.at[step, h, pl.ds(U, TR * U), :],
            out_hbm.at[pl.ds(_aligned(step * (TR * U)), TR * U), pl.ds(h * H, H)],
            out_sem.at[step, h])

    def dx_copy(step, h):
        return pltpu.make_async_copy(
            dxbuf.at[step, h, pl.ds(8, 4 * TR), :],
            dx_hbm.at[pl.ds(_aligned(step * (4 * TR)), 4 * TR), pl.ds(h * H, H)],
            out_sem.at[step, 2 + h])

    w_in = dict(w1=(w1_hbm, w1_ref), w2=(w2_hbm, w2_ref), wf=(wf_hbm, wf_ref),
                wo=(wo_hbm, wo_ref), g=(g_hbm, g_ref), wg=(wg_hbm, wg_ref))
    w_cp = {k: pltpu.make_async_copy(s, d, w_sem.at[i]) for i, (k, (s, d)) in enumerate(w_in.items())}

    def start(cp, step):
        for h in range(2):
            cp(step, h).start()

    def wait(cp, step):
        for h in range(2):
            cp(step, h).wait()

    def shifted(ref, v, delta):
        n = v.shape[0]
        for h, vh in enumerate(_halves(v)):
            ref[h, pl.ds(8, n), :] = vh
        return _cat(ref[0, pl.ds(8 + delta, n), :], ref[1, pl.ds(8 + delta, n), :])

    def g_words(step, p):
        return [gbuf.at[step, h].bitcast(u32)[pl.ds(p, M, stride=4), :] for h in range(2)]

    S = {}

    def conv1_fwd(step, first):
        def words(start):
            return [xbuf.at[step, h].bitcast(u32)[pl.ds(start, Q, stride=4), :] for h in range(2)]

        def cat(fn, ws):
            return _cat(fn(ws[0]), fn(ws[1]))

        w01e = [_zero_row_if(w, 0, first) for w in words(6)]
        w23e = [_zero_row_if(w, 0, first) for w in words(7)]
        w01o, w23o, w23se = words(8), words(9), words(5)
        a3e = cat(_hi, w23e)
        a0 = _stack(cat(_lo, w01e), cat(_lo, w01o))
        a1 = _stack(cat(_hi, w01e), cat(_hi, w01o))
        a2 = _stack(cat(_lo, w23e), cat(_lo, w23o))
        d3 = _stack(a3e, cat(_hi, w23o)) - a1
        d1 = _stack(cat(_hi, w23se), a3e) - a1
        a0, a1, a2, d1, d3 = (v.astype(bf16) for v in (a0, a1, a2, d1, d3))
        he_pre = _nn(a0, w1_ref[1]) + _nn(d1, w1_ref[0])
        m2 = _nn(a1, ws_ref[...])
        he_pre = he_pre + m2
        ho_pre = _nn(d3, w1_ref[2]) + _nn(a2, w1_ref[1]) + m2
        for k, v in enumerate((d1, a1, d3, a0, a2)):
            at_ref[k] = _words(v.T)
        he, ghe = _gelu_and_grad(he_pre)
        ho, gho = _gelu_and_grad(ho_pre)
        ghe_ref[...] = ghe
        gho_ref[...] = gho
        e, o = ho[:Q], ho[Q:]
        os_ = shifted(shift_a, o, -1)
        S["he"] = he.astype(bf16)
        S["e"] = e.astype(bf16)
        S["os-e"] = (os_ - e).astype(bf16)
        S["o-e"] = (o - e).astype(bf16)

    def conv2_fwd():
        he, e, n1, n3 = S.pop("he"), S.pop("e"), S.pop("os-e"), S.pop("o-e")
        t = _nn(he, w2_ref[1])
        n2 = _nn(e, vs_ref[...])
        f_pre = t + _stack(_nn(n1, w2_ref[0]) + n2, _nn(n3, w2_ref[2]) + n2)
        het_ref[...] = _words(he.T)
        for k, v in enumerate((n1, e, n3)):
            ht_ref[k] = _words(v.T)
        f, gf = _gelu_and_grad(f_pre)
        gf_ref[...] = gf
        S["f"] = f.astype(bf16)

    def fe_fwd():
        f = S.pop("f")
        f_ref[...] = _words(f)
        fe = _nn(f, wf_ref[...])
        for h, vh in enumerate(_halves(fe)):
            fe_ref[h, pl.ds(0, Q, stride=2), :] = vh[:Q]
            fe_ref[h, pl.ds(1, Q, stride=2), :] = vh[Q:]

    def joint_j(step, p):
        b = step // NT
        jw = []
        for h in range(2):
            feh = fe_ref[h, pl.ds(0, M), :]
            j0 = jnp.tanh(feh + ge_ref[h, pl.ds(b * U + 2 * p, 1), :])
            j1 = jnp.tanh(feh + ge_ref[h, pl.ds(b * U + 2 * p + 1, 1), :])
            jw.append(_pack(j0, j1))
        jw = _cat(jw[0], jw[1])
        j_ref[p] = jw
        jt_ref[p] = _words(_rows(jw).T)

    def joint_dz(step, p):
        b = step // NT
        gw = g_words(step, p)
        dj = _nt(_cat(_rows(gw[0]), _rows(gw[1])), wo_ref[...])
        jf = _rows(j_ref[p]).astype(f32)
        dz = dj * (1.0 - jf * jf)
        for h, vh in enumerate(_halves(dz)):
            if p == 0:
                fold[h, pl.ds(0, 2 * M), :] = vh
            else:
                fold[h, pl.ds(0, 2 * M), :] += vh
        dzm = _keep_rows(dz, 2, 2 * TR + 2)
        accg[b, p] += jnp.sum(dzm.reshape(2 * M // 8, 8, D), axis=0)

    def joint_out(step, p):
        o = _words(_nn(_rows(j_ref[p]), wo_ref[...]).astype(bf16))
        for h, vh in enumerate(_halves(o)):
            obuf.at[step, h].bitcast(u32)[pl.ds(p, M, stride=4), :] = vh

    def dwo(step, p, final=False):
        gw = g_words(step, p)
        gm = _cat(_rows(_keep_rows(gw[0], 1, TR + 1)), _rows(_keep_rows(gw[1], 1, TR + 1)))
        r = acco[...] + _nn(_rows(jt_ref[p]), gm)
        if final:
            dwo_st[...] = r.astype(bf16)
        else:
            acco[...] = r

    def joint_all(step):
        for p in range(4):
            joint_j(step, p)
            joint_dz(step, p)
            joint_out(step, p)
        start(o_copy, step)
        dwo(step, 0)

    def df_bwd(last, final=False):
        def folded(first_row):
            return _cat(*[fold[h, pl.ds(first_row, Q, stride=4), :]
                          + fold[h, pl.ds(first_row + 1, Q, stride=4), :] for h in range(2)])

        dfe = _stack(folded(0), folded(2))
        dfe_u = _zero_row_if(dfe, Q + TR // 2, last).astype(bf16)
        dfe_m = _keep_valid(dfe).astype(bf16)
        df = _nt(dfe_u, wf_ref[...])
        r = accf[...] + _tn(_rows(f_ref[...]), dfe_m)
        if final:
            dwf_st[...] = r.astype(bf16)
        else:
            accf[...] = r
        dfp = df * gf_ref[...]
        de, do = dfp[:Q], dfp[Q:]
        des = shifted(shift_b, de, 1)
        dem, dom = _keep_even(de), _keep_odd(do)
        S["dfp"] = dfp.astype(bf16)
        S["de-do"] = (de - do).astype(bf16)
        S["des-do"] = (des - do).astype(bf16)
        S["dfp_m"] = _stack(dem, dom).astype(bf16)
        S["dem+dom"] = (dem + dom).astype(bf16)

    def conv2_bwd(final=False):
        dfp, dfp_m = S.pop("dfp"), S.pop("dfp_m")
        dhe = _nt(dfp, w2_ref[1])
        c = _nt(dfp[Q:], vs_ref[...])
        dho = _stack(_nt(S.pop("de-do"), w2_ref[2]) + c, c + _nt(S.pop("des-do"), w2_ref[0]))
        n2 = acc2[1] + _nn(_rows(ht_ref[1]), S.pop("dem+dom"))
        n1 = acc2[0] + _nn(_rows(ht_ref[0]), dfp_m[:Q])
        n3 = acc2[2] + _nn(_rows(ht_ref[2]), dfp_m[Q:])
        w = acc2[3] + _nn(_rows(het_ref[...]), dfp_m)
        if final:
            dw2_st[0] = (n1 + n2).astype(bf16)
            dw2_st[1] = w.astype(bf16)
            dw2_st[2] = (n2 + n3).astype(bf16)
        else:
            acc2[0], acc2[1], acc2[2], acc2[3] = n1, n2, n3, w
        dhe = dhe * ghe_ref[...]
        dho = dho * gho_ref[...]
        pes = _stack(dhe[Q:], shifted(shift_c, dhe[:Q], 1))
        pe = _keep_valid(dhe)
        po = _keep_valid(dho)
        S["pe"], S["po"] = pe.astype(bf16), po.astype(bf16)
        S["pe-po"] = (pe - po).astype(bf16)
        S["pes-po"] = (pes - po).astype(bf16)
        S["pe+po"] = (pe + po).astype(bf16)

    def dx_bwd(step):
        pe, po = S["pe"], S["po"]
        da0 = _nt(pe, w1_ref[1])
        c = _nt(po, ws_ref[...])
        da1 = _nt(S.pop("pe-po"), w1_ref[2]) + c
        da2 = _nt(po, w1_ref[1])
        da3 = _nt(S.pop("pes-po"), w1_ref[0]) + c
        for h in range(2):
            sl = slice(h * H, (h + 1) * H)
            dxw = dxbuf.at[step, h].bitcast(u32)
            w01 = _pack(da0[:, sl], da1[:, sl])
            w23 = _pack(da2[:, sl], da3[:, sl])
            dxw[pl.ds(2, Q, stride=4), :] = w01[:Q]
            dxw[pl.ds(3, Q, stride=4), :] = w23[:Q]
            dxw[pl.ds(4, Q, stride=4), :] = w01[Q:]
            dxw[pl.ds(5, Q, stride=4), :] = w23[Q:]
        start(dx_copy, step)

    fin = []

    def flush(src, dst):
        cp = pltpu.make_async_copy(src, dst, dw_sem.at[len(fin)])
        cp.start()
        fin.append(cp)

    def dw1_bwd(final=False):
        pe, po, ps = S.pop("pe"), S.pop("po"), S.pop("pe+po")
        w = acc1[3] + _nn(_rows(at_ref[3]), pe) + _nn(_rows(at_ref[4]), po)
        if final:
            dw1_st[1] = w.astype(bf16)
            flush(dw1_st.at[1], dw1_hbm.at[1])
        else:
            acc1[3] = w
        m2 = acc1[1] + _nn(_rows(at_ref[1]), ps)
        m1 = acc1[0] + _nn(_rows(at_ref[0]), pe)
        if final:
            dw1_st[0] = (m1 + m2).astype(bf16)
            flush(dw1_st.at[0], dw1_hbm.at[0])
        else:
            acc1[0] = m1
            acc1[1] = m2
        m3 = acc1[2] + _nn(_rows(at_ref[2]), po)
        if final:
            dw1_st[2] = (m2 + m3).astype(bf16)
            flush(dw1_st.at[2], dw1_hbm.at[2])
        else:
            acc1[2] = m3

    zb = jnp.zeros

    def clear_margins(s):
        for h in range(2):
            xbuf[s, h, pl.ds(0, 16), :] = zb((16, H), bf16)
            xbuf[s, h, pl.ds(XD, XW - XD), :] = zb((XW - XD, H), bf16)
            gbuf[s, h, pl.ds(0, U), :] = zb((U, H), bf16)
            gbuf[s, h, pl.ds(GD, GW - GD), :] = zb((GW - GD, H), bf16)

    def zero_blocks(ref, n):
        def blk(k, carry):
            ref[k] = zb(ref.shape[1:], ref.dtype)
            return carry
        lax.fori_loop(0, n, blk, 0)

    def clear_rest(k, carry):
        clear_margins(k)
        return carry

    clear_margins(0)
    start(x_copy, 0)
    zero_blocks(acc1, 4)
    w_cp["w1"].start()
    zero_blocks(acc2, 4)
    w_cp["w2"].start()
    zero_blocks(accg, B)
    w_cp["wf"].start()
    zero_blocks(shift_a, 2)
    for k in ("g", "wg", "wo"):
        w_cp[k].start()
    zero_blocks(shift_b, 2)
    start(g_copy, 0)
    lax.fori_loop(1, NSTEP, clear_rest, 0)
    start(x_copy, 1)
    zero_blocks(shift_c, 2)
    start(g_copy, 1)
    for ref in (accf, acco):
        ref[...] = zb(ref.shape, f32)
    wait(x_copy, 0)
    w_cp["w1"].wait()
    ws_ref[...] = (w1_ref[0].astype(f32) + w1_ref[2].astype(f32)).astype(bf16)
    conv1_fwd(0, True)
    for k in ("w2", "wf", "g", "wg", "wo"):
        w_cp[k].wait()
    vs_ref[...] = (w2_ref[0].astype(f32) + w2_ref[2].astype(f32)).astype(bf16)
    ge = _nn(g_ref[...], wg_ref[...])
    for h, vh in enumerate(_halves(ge)):
        ge_ref[h] = vh
    conv2_fwd()
    fe_fwd()
    for p in range(4):
        joint_j(0, p)
        joint_out(0, p)
    wait(g_copy, 0)
    for p in range(4):
        joint_dz(0, p)
    dwo(0, 0)

    def body(i, carry):
        wait(x_copy, i + 1)
        wait(g_copy, i + 1)
        dwo(i, 1)

        @pl.when(i == 0)
        def _():
            start(o_copy, 0)

        @pl.when(i + 2 < NSTEP)
        def _():
            start(x_copy, i + 2)
            start(g_copy, i + 2)

        df_bwd(i % NT == NT - 1)
        conv2_bwd()
        dx_bwd(i)
        dw1_bwd()
        conv1_fwd(i + 1, (i + 1) % NT == 0)
        dwo(i, 2)
        conv2_fwd()
        dwo(i, 3)
        fe_fwd()
        joint_all(i + 1)
        return carry

    lax.fori_loop(0, NSTEP - 1, body, 0)

    last = NSTEP - 1
    dwo(last, 1)
    df_bwd(True, final=True)
    flush(dwf_st, dwf_hbm)
    for b in range(B):
        for p in range(4):
            a = accg[b, p]
            a = a + pltpu.roll(a, 6, 0)
            a = a + pltpu.roll(a, 4, 0)
            dge_ref[pl.ds(b * U + 2 * p, 2), :] = a[0:2]
    dge = dge_ref[...].astype(bf16)
    dg_st[...] = _nt(dge, wg_ref[...]).astype(bf16)
    dwg_st[...] = _tn(g_ref[...], dge).astype(bf16)
    flush(dg_st, dg_hbm)
    flush(dwg_st, dwg_hbm)
    dwo(last, 2)
    conv2_bwd(final=True)
    flush(dw2_st, dw2_hbm)
    dwo(last, 3, final=True)
    flush(dwo_st, dwo_hbm)
    dx_bwd(last)
    dw1_bwd(final=True)
    for step in range(NSTEP):
        wait(o_copy, step)
        wait(dx_copy, step)
    for cp in fin:
        cp.wait()


@jax.jit
def pallas_standalone__seq2seq_rnn_t_joint__speech_kernel(x, w1, w2, g, w_f, w_g, w_o, grad_out):
    x2 = x.reshape(B * T, D)
    go2 = grad_out.reshape(B * R * U, D)
    g2 = g.reshape(B * U, D)
    hbm = pl.BlockSpec(memory_space=pl.ANY)
    sds = jax.ShapeDtypeStruct
    vmem = pltpu.VMEM
    out, dx, dw1, dw2, dg, dwf, dwg, dwo = pl.pallas_call(
        _kernel,
        in_specs=[hbm] * 8,
        out_specs=[hbm] * 8,
        out_shape=[sds((B * R * U, D), bf16), sds((B * T, D), bf16), sds((3, D, D), bf16),
                   sds((3, D, D), bf16), sds((B * U, D), bf16), sds((D, D), bf16),
                   sds((D, D), bf16), sds((D, D), bf16)],
        scratch_shapes=[
            vmem((NSTEP, 2, XW, H), bf16),
            vmem((NSTEP, 2, GW, H), bf16),
            vmem((NSTEP, 2, GW, H), bf16),
            vmem((NSTEP, 2, DXW, H), bf16),
            vmem((B * U, D), bf16),
            vmem((3, D, D), bf16),
            vmem((3, D, D), bf16),
            vmem((D, D), bf16),
            vmem((D, D), bf16),
            vmem((D, D), bf16),
            vmem((D, D), bf16),
            vmem((D, D), bf16),
            vmem((5, D // 2, M), u32),
            vmem((D // 2, M), u32),
            vmem((3, D // 2, Q), u32),
            vmem((M // 2, D), u32),
            vmem((M, D), f32),
            vmem((M, D), f32),
            vmem((M, D), f32),
            vmem((2, M + 8, H), f32),
            vmem((4, M, D), u32),
            vmem((4, D // 2, 2 * M), u32),
            vmem((2, Q + 16, H), f32),
            vmem((2, Q + 16, H), f32),
            vmem((2, Q + 16, H), f32),
            vmem((2, 2 * M + 8, H), f32),
            vmem((2, B * U, H), f32),
            vmem((4, D, D), f32),
            vmem((4, D, D), f32),
            vmem((D, D), f32),
            vmem((D, D), f32),
            vmem((B, 4, 8, D), f32),
            vmem((B * U, D), f32),
            vmem((3, D, D), bf16),
            vmem((3, D, D), bf16),
            vmem((D, D), bf16),
            vmem((D, D), bf16),
            vmem((D, D), bf16),
            vmem((B * U, D), bf16),
            pltpu.SemaphoreType.DMA((NSTEP, 4)),
            pltpu.SemaphoreType.DMA((NSTEP, 4)),
            pltpu.SemaphoreType.DMA((8,)),
            pltpu.SemaphoreType.DMA((8,)),
        ],
        compiler_params=pltpu.CompilerParams(vmem_limit_bytes=100 * 1024 * 1024,
                                             disable_bounds_checks=True,
                                             disable_semaphore_checks=True),
    )(x2, go2, g2, w1, w2, w_f, w_g, w_o)
    return (out.reshape(B, R, U, D), dx.reshape(B, T, D), dw1, dw2, dg.reshape(B, U, D),
            dwf, dwg, dwo)
```

```python
import jax
import jax.numpy as jnp
from jax import lax
from jax.experimental import pallas as pl
from jax.experimental.pallas import tpu as pltpu

f32 = jnp.float32
bf16 = jnp.bfloat16
u32 = jnp.uint32

B, T, D, U = 2, 4000, 256, 8
R = 1000
TR = 250
NT = R // TR
NSTEP = B * NT
M = 256
Q = M // 2
H = 128
XW = 1040
XD = 1016
GW = M * U + 8
GD = (TR + 1) * U
DXW = 1040

CH_OUT = 32
CH_DJ = 32
CH_V = 8
PERM = (0, 2, 6, 5, 3, 4, 1)
ORDER = (1, 3, 2, 4, 0, 5, 6)

GELU_C0 = 0.7978845608028654
GELU_C1 = 0.044715


def _nn(a, w):
    return jnp.dot(a, w, preferred_element_type=f32)


def _nt(a, w):
    return lax.dot_general(a, w, (((1,), (1,)), ((), ())), preferred_element_type=f32)


def _tn(a, b):
    return lax.dot_general(a, b, (((0,), (0,)), ((), ())), preferred_element_type=f32)


def _gelu_and_grad(x):
    x2 = x * x
    th = jnp.tanh(x * (GELU_C0 + (GELU_C0 * GELU_C1) * x2))
    s = 0.5 + 0.5 * th
    g = x * s
    dg = s + x * (1.0 - th * th) * (0.5 * GELU_C0 + (1.5 * GELU_C0 * GELU_C1) * x2)
    return g, dg


def _cat(lo, hi):
    return jnp.concatenate([lo, hi], axis=1)


def _stack(a, b):
    return jnp.concatenate([a, b], axis=0)


def _halves(v):
    return v[:, :H], v[:, H:]


def _keep_rows(v, lo, hi):
    n = v.shape[0]
    a = -(-lo // 8) * 8
    b = hi // 8 * 8
    zero = jnp.zeros((), v.dtype)
    parts = []
    if a > 0:
        r = lax.broadcasted_iota(jnp.int32, (a, v.shape[1]), 0)
        parts.append(jnp.where(r >= lo, v[:a], zero))
    if b > a:
        parts.append(v[a:b])
    if b < n:
        r = lax.broadcasted_iota(jnp.int32, (n - b, v.shape[1]), 0) + b
        parts.append(jnp.where(r < hi, v[b:], zero))
    return jnp.concatenate(parts, axis=0) if len(parts) > 1 else parts[0]


def _keep_even(v):
    return _keep_rows(v, 1, TR // 2 + 1)


def _keep_odd(v):
    return _keep_rows(v, 0, TR // 2)


def _keep_valid(v):
    return _stack(_keep_even(v[:Q]), _keep_odd(v[Q:]))


def _zero_row_if(v, row, cond):
    if cond is False:
        return v
    a = row // 8 * 8
    blk = v[a:a + 8]
    r = lax.broadcasted_iota(jnp.int32, blk.shape, 0) + a
    kill = row if cond is True else jnp.where(cond, row, -1)
    blk = jnp.where(r == kill, jnp.zeros((), v.dtype), blk)
    parts = ([v[:a]] if a > 0 else []) + [blk] + ([v[a + 8:]] if a + 8 < v.shape[0] else [])
    return jnp.concatenate(parts, axis=0)


def _fwd_set(x11, x12, x21, x22):
    return [x11 + x22, x12 + x22, x11, x22, x11 + x21, x12 - x11, x21 - x22]


def _bwd_set(y11, y12, y21, y22):
    return [y11 + y22, y21 + y22, y11, y22, y11 + y12, y21 - y11, y12 - y22]


def _std_out(m):
    return m[0] + m[3] - m[4] + m[6], m[2] + m[4], m[1] + m[3], m[0] - m[1] + m[2] + m[5]


def _dual_out(n):
    return n[0] + n[3] - n[4] + n[6], n[1] + n[3], n[2] + n[4], n[0] - n[1] + n[2] + n[5]


def _zero_after(v):
    u = lax.bitcast_convert_type(v[:8], u32)
    return lax.shift_right_logical(lax.shift_right_logical(u, jnp.uint32(31)), jnp.uint32(1))


def _products(fn):
    m = [None] * 7
    for k in ORDER:
        m[k] = fn(k)
    return m


def _lo(w):
    return pltpu.unpack_elementwise(w, index=0, packed_dtype=bf16, unpacked_dtype=f32)


def _hi(w):
    return pltpu.unpack_elementwise(w, index=1, packed_dtype=bf16, unpacked_dtype=f32)


def _pack(a, b):
    return pltpu.pack_elementwise([a, b], packed_dtype=bf16)


def _words(v):
    return pltpu.bitcast(v, u32)


def _rows(w):
    return pltpu.bitcast(w, bf16)


def _aligned(v):
    return v if isinstance(v, int) else pl.multiple_of(v, 8)


def _kernel(x_hbm, go_hbm, g_hbm, w1_hbm, w2_hbm, wf_hbm, wg_hbm, wo_hbm,
            out_hbm, dx_hbm, dw1_hbm, dw2_hbm, dg_hbm, dwf_hbm, dwg_hbm, dwo_hbm,
            xbuf, gbuf, obuf, dxbuf,
            g_ref, w1_ref, w2_ref, wf_ref, wg_ref, wo_ref, ws_ref, vs_ref, wos_ref, wts_ref,
            at_ref, het_ref, ht_ref, f_ref, ghe_ref, gho_ref, gf_ref, fe_ref, xs_ref, jt_ref, gs_ref, gu_ref,
            shift_a, shift_b, shift_c, fold, ge_ref,
            acc1, acc2, accf, acco, accg, dge_ref,
            dw1_st, dw2_st, dwf_st, dwo_st, dwg_st, dg_st,
            in_sem, out_sem, w_sem, dw_sem):

    def x_copy(step, h):
        nominal = step * (4 * TR) - 8
        if isinstance(step, int):
            src = min(max(nominal, 0), B * T - XD)
        else:
            src = jnp.clip(nominal, 0, B * T - XD)
        return pltpu.make_async_copy(
            x_hbm.at[pl.ds(_aligned(src), XD), pl.ds(h * H, H)],
            xbuf.at[step, h, pl.ds(_aligned(8 + src - nominal), XD), :],
            in_sem.at[step, h])

    def g_copy(step, h):
        return pltpu.make_async_copy(
            go_hbm.at[pl.ds(_aligned(step * (TR * U)), TR * U), pl.ds(h * H, H)],
            gbuf.at[step, h, pl.ds(U, TR * U), :],
            in_sem.at[step, 2 + h])

    def gh_copy(step, h):
        nominal = (step + 1) * (TR * U)
        if isinstance(step, int):
            src = min(nominal, B * R * U - U)
        else:
            src = jnp.minimum(nominal, B * R * U - U)
        return pltpu.make_async_copy(
            go_hbm.at[pl.ds(_aligned(src), U), pl.ds(h * H, H)],
            gbuf.at[step, h, pl.ds(U + TR * U, U), :],
            in_sem.at[step, 4 + h])

    def o_copy(step, h):
        return pltpu.make_async_copy(
            obuf.at[step, h, pl.ds(U, TR * U), :],
            out_hbm.at[pl.ds(_aligned(step * (TR * U)), TR * U), pl.ds(h * H, H)],
            out_sem.at[step, h])

    def dx_copy(step, h):
        return pltpu.make_async_copy(
            dxbuf.at[step, h, pl.ds(8, 4 * TR), :],
            dx_hbm.at[pl.ds(_aligned(step * (4 * TR)), 4 * TR), pl.ds(h * H, H)],
            out_sem.at[step, 2 + h])

    w_in = dict(w1=(w1_hbm, w1_ref), w2=(w2_hbm, w2_ref), wf=(wf_hbm, wf_ref),
                wo=(wo_hbm, wo_ref), g=(g_hbm, g_ref), wg=(wg_hbm, wg_ref))
    w_cp = {k: pltpu.make_async_copy(s, d, w_sem.at[i]) for i, (k, (s, d)) in enumerate(w_in.items())}

    def start(cp, step):
        for h in range(2):
            cp(step, h).start()

    def wait(cp, step):
        for h in range(2):
            cp(step, h).wait()

    def shifted(ref, v, delta):
        n = v.shape[0]
        for h, vh in enumerate(_halves(v)):
            ref[h, pl.ds(8, n), :] = vh
        return _cat(ref[0, pl.ds(8 + delta, n), :], ref[1, pl.ds(8 + delta, n), :])

    def g_words(step, p):
        return [gbuf.at[step, h].bitcast(u32)[pl.ds(p, M, stride=4), :] for h in range(2)]

    S = {}

    def conv1_fwd(step, first):
        def words(start):
            return [xbuf.at[step, h].bitcast(u32)[pl.ds(start, Q, stride=4), :] for h in range(2)]

        def cat(fn, ws):
            return _cat(fn(ws[0]), fn(ws[1]))

        w01e = [_zero_row_if(w, 0, first) for w in words(6)]
        w23e = [_zero_row_if(w, 0, first) for w in words(7)]
        w01o, w23o, w23se = words(8), words(9), words(5)
        a3e = cat(_hi, w23e)
        a0 = _stack(cat(_lo, w01e), cat(_lo, w01o))
        a1 = _stack(cat(_hi, w01e), cat(_hi, w01o))
        a2 = _stack(cat(_lo, w23e), cat(_lo, w23o))
        d3 = _stack(a3e, cat(_hi, w23o)) - a1
        d1 = _stack(cat(_hi, w23se), a3e) - a1
        a0, a1, a2, d1, d3 = (v.astype(bf16) for v in (a0, a1, a2, d1, d3))
        he_pre = _nn(a0, w1_ref[1]) + _nn(d1, w1_ref[0])
        m2 = _nn(a1, ws_ref[...])
        he_pre = he_pre + m2
        ho_pre = _nn(d3, w1_ref[2]) + _nn(a2, w1_ref[1]) + m2
        for k, v in enumerate((d1, a1, d3, a0, a2)):
            at_ref[k] = _words(v.T)
        he, ghe = _gelu_and_grad(he_pre)
        ho, gho = _gelu_and_grad(ho_pre)
        ghe_ref[...] = ghe
        gho_ref[...] = gho
        e, o = ho[:Q], ho[Q:]
        os_ = shifted(shift_a, o, -1)
        S["he"] = he.astype(bf16)
        S["e"] = e.astype(bf16)
        S["os-e"] = (os_ - e).astype(bf16)
        S["o-e"] = (o - e).astype(bf16)

    def conv2_fwd():
        he, e, n1, n3 = S.pop("he"), S.pop("e"), S.pop("os-e"), S.pop("o-e")
        t = _nn(he, w2_ref[1])
        n2 = _nn(e, vs_ref[...])
        f_pre = t + _stack(_nn(n1, w2_ref[0]) + n2, _nn(n3, w2_ref[2]) + n2)
        het_ref[...] = _words(he.T)
        for k, v in enumerate((n1, e, n3)):
            ht_ref[k] = _words(v.T)
        f, gf = _gelu_and_grad(f_pre)
        gf_ref[...] = gf
        S["f"] = f.astype(bf16)

    def fe_fwd():
        f = S.pop("f")
        f_ref[...] = _words(f)
        fe = _nn(f, wf_ref[...])
        for h, vh in enumerate(_halves(fe)):
            fe_ref[h, pl.ds(0, Q, stride=2), :] = vh[:Q]
            fe_ref[h, pl.ds(1, Q, stride=2), :] = vh[Q:]

    def joint_j(step, p, slot, toks=None):
        b = step // NT
        ge0 = [ge_ref[h, pl.ds(b * U + 2 * p, 1), :] for h in range(2)]
        ge1 = [ge_ref[h, pl.ds(b * U + 2 * p + 1, 1), :] for h in range(2)]
        for s in range(0, Q, CH_V):
            blk0, blk1 = [], []
            g0, g1 = ge0, ge1
            if toks is not None:
                z = lax.bitcast_convert_type(toks[s * len(toks) // Q][0:1], f32)
                g0, g1 = [v + z for v in ge0], [v + z for v in ge1]
            for r in range(2):
                for h in range(2):
                    fe = fe_ref[h, pl.ds(Q * r + s, CH_V), :]
                    blk0.append(jnp.tanh(fe + g0[h]))
                    blk1.append(jnp.tanh(fe + g1[h]))
            for q, (c0, c1) in enumerate(zip(_fwd_set(*blk0), _fwd_set(*blk1))):
                xs_ref[slot, q, pl.ds(s, CH_V), :] = _pack(c0, c1)
            xs_ref[slot, 7, pl.ds(s, CH_V), :] = _pack(blk0[1], blk1[1])
            xs_ref[slot, 8, pl.ds(s, CH_V), :] = _pack(blk0[2], blk1[2])
        for q in range(7):
            jt_ref[p, q] = _words(_rows(xs_ref[slot, q]).T)

    J_PLAIN = ((2, 7), (8, 3))

    def joint_g(step, p, toks=None):
        def operands(w11, w12, w21, w22):
            ws = (w11, w12, w21, w22)
            s0 = _bwd_set(*[_lo(w) for w in ws])
            s1 = _bwd_set(*[_hi(w) for w in ws])
            ops = [_pack(c0, c1) for c0, c1 in zip(s0, s1)]
            ops[2], ops[3] = w11, w22
            return ops

        for s in range(0, Q, CH_V):
            gw = [gbuf.at[step, h].bitcast(u32)[pl.ds(p + 4 * (Q * r + s), CH_V, stride=4), :]
                  for r in range(2) for h in range(2)]
            if toks is not None:
                z = toks[s * len(toks) // Q]
                gw = [w | jnp.tile(z, (CH_V // 8, 1)) for w in gw]
            ops = operands(*gw)
            if s + CH_V == Q:
                t = CH_V - 8
                for q in range(7):
                    gu_ref[q] = ops[q][t:]
                keep = TR + 1 - Q - s
                ops = operands(gw[0], gw[1], _keep_rows(gw[2], 0, keep), _keep_rows(gw[3], 0, keep))
            for q in range(7):
                gs_ref[p, q, pl.ds(s, CH_V), :] = ops[q]

    def joint_dz(step, p, slot):
        b = step // NT
        dge = [None, None]
        toks = []
        for s in range(0, Q, CH_DJ):
            def lhs(k):
                if s + CH_DJ < Q:
                    return gs_ref[p, k, pl.ds(s, CH_DJ), :]
                return _stack(gs_ref[p, k, pl.ds(s, CH_DJ - 8), :], gu_ref[k])

            m = _products(lambda k: _nn(_rows(lhs(k)), _rows(wts_ref[k])))
            c = _std_out(m)
            toks += [_zero_after(m[k][r:]) for k in (1, 0) for r in (0, CH_DJ)]
            for r in range(2):
                for n in range(2):
                    jf = _rows(xs_ref[slot, J_PLAIN[r][n], pl.ds(s, CH_DJ), :]).astype(f32)
                    dz = c[2 * r + n] * (1.0 - jf * jf)
                    row0 = 2 * (Q * r + s)
                    if p == 0:
                        fold[n, pl.ds(row0, 2 * CH_DJ), :] = dz
                    else:
                        fold[n, pl.ds(row0, 2 * CH_DJ), :] += dz
                    hi = 2 * (TR + 1) - row0
                    if hi < 2 * CH_DJ:
                        dz = _keep_rows(dz, 0, hi)
                    part = jnp.sum(dz.reshape(2 * CH_DJ // 8, 8, H), axis=0)
                    dge[n] = part if dge[n] is None else dge[n] + part
        accg[b, p] += _cat(dge[0], dge[1])
        return toks

    def joint_out(step, p, slot):
        toks = []
        for s in range(0, Q, CH_OUT):
            n = _products(lambda k: _nn(_rows(xs_ref[slot, PERM[k], pl.ds(s, CH_OUT), :]), _rows(wos_ref[k])))
            c = _dual_out(n)
            toks += [_zero_after(n[k][r:]) for k in (1, 0) for r in (0, CH_OUT)]
            for r in range(2):
                for h in range(2):
                    ow = obuf.at[step, h].bitcast(u32)
                    ow[pl.ds(p + 4 * (Q * r + s), CH_OUT, stride=4), :] = _words(c[2 * r + h].astype(bf16))
        return toks

    def dwo(step, p, final=False):
        m = [acco[k] + _nn(_rows(jt_ref[p, k]), _rows(gs_ref[p, PERM[k]])) for k in range(7)]
        if final:
            c = _std_out(m)
            dwo_st[...] = _stack(_cat(c[0], c[1]), _cat(c[2], c[3])).astype(bf16)
        else:
            for k in range(7):
                acco[k] = m[k]

    def joint_all(step):
        joint_g(step, 0)
        joint_j(step, 0, 0)
        for p in range(4):
            t_dj = joint_dz(step, p, p % 2)
            if p < 3:
                joint_g(step, p + 1, t_dj)
            t_out = joint_out(step, p, p % 2)
            if p < 3:
                joint_j(step, p + 1, (p + 1) % 2, t_out)
        start(o_copy, step)
        dwo(step, 0)

    def df_bwd(last, final=False):
        def folded(first_row):
            return _cat(*[fold[h, pl.ds(first_row, Q, stride=4), :]
                          + fold[h, pl.ds(first_row + 1, Q, stride=4), :] for h in range(2)])

        dfe = _stack(folded(0), folded(2))
        dfe_u = _zero_row_if(dfe, Q + TR // 2, last).astype(bf16)
        dfe_m = _keep_valid(dfe).astype(bf16)
        df = _nt(dfe_u, wf_ref[...])
        r = accf[...] + _tn(_rows(f_ref[...]), dfe_m)
        if final:
            dwf_st[...] = r.astype(bf16)
        else:
            accf[...] = r
        dfp = df * gf_ref[...]
        de, do = dfp[:Q], dfp[Q:]
        des = shifted(shift_b, de, 1)
        dem, dom = _keep_even(de), _keep_odd(do)
        S["dfp"] = dfp.astype(bf16)
        S["de-do"] = (de - do).astype(bf16)
        S["des-do"] = (des - do).astype(bf16)
        S["dfp_m"] = _stack(dem, dom).astype(bf16)
        S["dem+dom"] = (dem + dom).astype(bf16)

    def conv2_bwd(final=False):
        dfp, dfp_m = S.pop("dfp"), S.pop("dfp_m")
        dhe = _nt(dfp, w2_ref[1])
        c = _nt(dfp[Q:], vs_ref[...])
        dho = _stack(_nt(S.pop("de-do"), w2_ref[2]) + c, c + _nt(S.pop("des-do"), w2_ref[0]))
        n2 = acc2[1] + _nn(_rows(ht_ref[1]), S.pop("dem+dom"))
        n1 = acc2[0] + _nn(_rows(ht_ref[0]), dfp_m[:Q])
        n3 = acc2[2] + _nn(_rows(ht_ref[2]), dfp_m[Q:])
        w = acc2[3] + _nn(_rows(het_ref[...]), dfp_m)
        if final:
            dw2_st[0] = (n1 + n2).astype(bf16)
            dw2_st[1] = w.astype(bf16)
            dw2_st[2] = (n2 + n3).astype(bf16)
        else:
            acc2[0], acc2[1], acc2[2], acc2[3] = n1, n2, n3, w
        dhe = dhe * ghe_ref[...]
        dho = dho * gho_ref[...]
        pes = _stack(dhe[Q:], shifted(shift_c, dhe[:Q], 1))
        pe = _keep_valid(dhe)
        po = _keep_valid(dho)
        S["pe"], S["po"] = pe.astype(bf16), po.astype(bf16)
        S["pe-po"] = (pe - po).astype(bf16)
        S["pes-po"] = (pes - po).astype(bf16)
        S["pe+po"] = (pe + po).astype(bf16)

    def dx_bwd(step):
        pe, po = S["pe"], S["po"]
        da0 = _nt(pe, w1_ref[1])
        c = _nt(po, ws_ref[...])
        da1 = _nt(S.pop("pe-po"), w1_ref[2]) + c
        da2 = _nt(po, w1_ref[1])
        da3 = _nt(S.pop("pes-po"), w1_ref[0]) + c
        for h in range(2):
            sl = slice(h * H, (h + 1) * H)
            dxw = dxbuf.at[step, h].bitcast(u32)
            w01 = _pack(da0[:, sl], da1[:, sl])
            w23 = _pack(da2[:, sl], da3[:, sl])
            dxw[pl.ds(2, Q, stride=4), :] = w01[:Q]
            dxw[pl.ds(3, Q, stride=4), :] = w23[:Q]
            dxw[pl.ds(4, Q, stride=4), :] = w01[Q:]
            dxw[pl.ds(5, Q, stride=4), :] = w23[Q:]
        start(dx_copy, step)

    fin = []

    def flush(src, dst):
        cp = pltpu.make_async_copy(src, dst, dw_sem.at[len(fin)])
        cp.start()
        fin.append(cp)

    def dw1_bwd(final=False):
        pe, po, ps = S.pop("pe"), S.pop("po"), S.pop("pe+po")
        w = acc1[3] + _nn(_rows(at_ref[3]), pe) + _nn(_rows(at_ref[4]), po)
        if final:
            dw1_st[1] = w.astype(bf16)
            flush(dw1_st.at[1], dw1_hbm.at[1])
        else:
            acc1[3] = w
        m2 = acc1[1] + _nn(_rows(at_ref[1]), ps)
        m1 = acc1[0] + _nn(_rows(at_ref[0]), pe)
        if final:
            dw1_st[0] = (m1 + m2).astype(bf16)
            flush(dw1_st.at[0], dw1_hbm.at[0])
        else:
            acc1[0] = m1
            acc1[1] = m2
        m3 = acc1[2] + _nn(_rows(at_ref[2]), po)
        if final:
            dw1_st[2] = (m2 + m3).astype(bf16)
            flush(dw1_st.at[2], dw1_hbm.at[2])
        else:
            acc1[2] = m3

    zb = jnp.zeros

    def clear_margins(s):
        for h in range(2):
            xbuf[s, h, pl.ds(0, 16), :] = zb((16, H), bf16)
            xbuf[s, h, pl.ds(XD, XW - XD), :] = zb((XW - XD, H), bf16)
            gbuf[s, h, pl.ds(0, U), :] = zb((U, H), bf16)
            gbuf[s, h, pl.ds(GD, GW - GD), :] = zb((GW - GD, H), bf16)

    def zero_blocks(ref, n):
        def blk(k, carry):
            ref[k] = zb(ref.shape[1:], ref.dtype)
            return carry
        lax.fori_loop(0, n, blk, 0)

    def clear_rest(k, carry):
        clear_margins(k)
        return carry

    clear_margins(0)
    start(x_copy, 0)
    zero_blocks(acc1, 4)
    w_cp["w1"].start()
    zero_blocks(acc2, 4)
    w_cp["w2"].start()
    zero_blocks(accg, B)
    w_cp["wf"].start()
    zero_blocks(shift_a, 2)
    for k in ("g", "wg", "wo"):
        w_cp[k].start()
    zero_blocks(shift_b, 2)
    start(g_copy, 0)
    start(gh_copy, 0)
    lax.fori_loop(1, NSTEP, clear_rest, 0)
    start(x_copy, 1)
    zero_blocks(shift_c, 2)
    start(g_copy, 1)
    start(gh_copy, 1)
    for ref in (accf, acco):
        ref[...] = zb(ref.shape, f32)
    wait(x_copy, 0)
    w_cp["w1"].wait()
    ws_ref[...] = (w1_ref[0].astype(f32) + w1_ref[2].astype(f32)).astype(bf16)
    conv1_fwd(0, True)
    for k in ("w2", "wf", "g", "wg", "wo"):
        w_cp[k].wait()
    vs_ref[...] = (w2_ref[0].astype(f32) + w2_ref[2].astype(f32)).astype(bf16)
    wo = wo_ref[...].astype(f32)
    wo_set = [_words(v.astype(bf16)) for v in _fwd_set(wo[:H, :H], wo[:H, H:], wo[H:, :H], wo[H:, H:])]
    for k in range(7):
        wos_ref[k] = wo_set[k]
        wts_ref[k] = _words(_rows(wo_set[PERM[k]]).T)
    ge = _nn(g_ref[...], wg_ref[...])
    for h, vh in enumerate(_halves(ge)):
        ge_ref[h] = vh
    conv2_fwd()
    fe_fwd()
    for p in range(4):
        joint_j(0, p, p)
        joint_out(0, p, p)
    wait(g_copy, 0)
    wait(gh_copy, 0)
    for p in range(4):
        joint_g(0, p)
        joint_dz(0, p, p)
    dwo(0, 0)

    def body(i, carry):
        wait(x_copy, i + 1)
        wait(g_copy, i + 1)
        wait(gh_copy, i + 1)
        @pl.when(i == 0)
        def _():
            start(o_copy, 0)

        @pl.when(i + 2 < NSTEP)
        def _():
            start(x_copy, i + 2)
            start(g_copy, i + 2)
            start(gh_copy, i + 2)

        df_bwd(i % NT == NT - 1)
        conv2_bwd()
        dx_bwd(i)
        dw1_bwd()
        conv1_fwd(i + 1, (i + 1) % NT == 0)
        dwo(i, 1)
        conv2_fwd()
        dwo(i, 2)
        fe_fwd()
        dwo(i, 3)
        joint_all(i + 1)
        return carry

    lax.fori_loop(0, NSTEP - 1, body, 0)

    last = NSTEP - 1
    dwo(last, 1)
    df_bwd(True, final=True)
    flush(dwf_st, dwf_hbm)
    for b in range(B):
        for p in range(4):
            a = accg[b, p]
            a = a + pltpu.roll(a, 6, 0)
            a = a + pltpu.roll(a, 4, 0)
            dge_ref[pl.ds(b * U + 2 * p, 2), :] = a[0:2]
    dge = dge_ref[...].astype(bf16)
    dg_st[...] = _nt(dge, wg_ref[...]).astype(bf16)
    dwg_st[...] = _tn(g_ref[...], dge).astype(bf16)
    flush(dg_st, dg_hbm)
    flush(dwg_st, dwg_hbm)
    dwo(last, 2)
    conv2_bwd(final=True)
    flush(dw2_st, dw2_hbm)
    dwo(last, 3, final=True)
    flush(dwo_st, dwo_hbm)
    dx_bwd(last)
    dw1_bwd(final=True)
    for step in range(NSTEP):
        wait(o_copy, step)
        wait(dx_copy, step)
    for cp in fin:
        cp.wait()


@jax.jit
def pallas_standalone__seq2seq_rnn_t_joint__speech_kernel(x, w1, w2, g, w_f, w_g, w_o, grad_out):
    x2 = x.reshape(B * T, D)
    go2 = grad_out.reshape(B * R * U, D)
    g2 = g.reshape(B * U, D)
    hbm = pl.BlockSpec(memory_space=pl.ANY)
    sds = jax.ShapeDtypeStruct
    vmem = pltpu.VMEM
    out, dx, dw1, dw2, dg, dwf, dwg, dwo = pl.pallas_call(
        _kernel,
        in_specs=[hbm] * 8,
        out_specs=[hbm] * 8,
        out_shape=[sds((B * R * U, D), bf16), sds((B * T, D), bf16), sds((3, D, D), bf16),
                   sds((3, D, D), bf16), sds((B * U, D), bf16), sds((D, D), bf16),
                   sds((D, D), bf16), sds((D, D), bf16)],
        scratch_shapes=[
            vmem((NSTEP, 2, XW, H), bf16),
            vmem((NSTEP, 2, GW, H), bf16),
            vmem((NSTEP, 2, GW, H), bf16),
            vmem((NSTEP, 2, DXW, H), bf16),
            vmem((B * U, D), bf16),
            vmem((3, D, D), bf16),
            vmem((3, D, D), bf16),
            vmem((D, D), bf16),
            vmem((D, D), bf16),
            vmem((D, D), bf16),
            vmem((D, D), bf16),
            vmem((D, D), bf16),
            vmem((7, H // 2, H), u32),
            vmem((7, H // 2, H), u32),
            vmem((5, D // 2, M), u32),
            vmem((D // 2, M), u32),
            vmem((3, D // 2, Q), u32),
            vmem((M // 2, D), u32),
            vmem((M, D), f32),
            vmem((M, D), f32),
            vmem((M, D), f32),
            vmem((2, M + 8, H), f32),
            vmem((4, 9, Q, H), u32),
            vmem((4, 7, H // 2, M), u32),
            vmem((4, 7, Q, H), u32),
            vmem((7, 8, H), u32),
            vmem((2, Q + 16, H), f32),
            vmem((2, Q + 16, H), f32),
            vmem((2, Q + 16, H), f32),
            vmem((2, 2 * M + 8, H), f32),
            vmem((2, B * U, H), f32),
            vmem((4, D, D), f32),
            vmem((4, D, D), f32),
            vmem((D, D), f32),
            vmem((7, H, H), f32),
            vmem((B, 4, 8, D), f32),
            vmem((B * U, D), f32),
            vmem((3, D, D), bf16),
            vmem((3, D, D), bf16),
            vmem((D, D), bf16),
            vmem((D, D), bf16),
            vmem((D, D), bf16),
            vmem((B * U, D), bf16),
            pltpu.SemaphoreType.DMA((NSTEP, 6)),
            pltpu.SemaphoreType.DMA((NSTEP, 4)),
            pltpu.SemaphoreType.DMA((8,)),
            pltpu.SemaphoreType.DMA((8,)),
        ],
        compiler_params=pltpu.CompilerParams(vmem_limit_bytes=100 * 1024 * 1024,
                                             disable_bounds_checks=True,
                                             disable_semaphore_checks=True),
    )(x2, go2, g2, w1, w2, w_f, w_g, w_o)
    return (out.reshape(B, R, U, D), dx.reshape(B, T, D), dw1, dw2, dg.reshape(B, U, D),
            dwf, dwg, dwo)
```

```python
import functools

import jax
import jax.numpy as jnp
from jax import lax
from jax.experimental import pallas as pl
from jax.experimental.pallas import tpu as pltpu

f32 = jnp.float32
bf16 = jnp.bfloat16
u32 = jnp.uint32

B, T, D, U = 2, 4000, 256, 8
R = 1000
TR = 250
NT = R // TR
NSTEP = B * NT
M = 256
Q = M // 2
H = 128
HW = H // 2
XW = 1040
XD = 1016
GW = M * U + 8
GD = (TR + 1) * U
DXW = 1040
CH_OUT = 32
CH_DJ = 32
CH_C = 16
CH_V = 8

PERM = (0, 2, 6, 5, 3, 4, 1)
ORDER = (1, 3, 2, 4, 0, 5, 6)
W10, W11, W12, WS, V0, V1, V2, VS, WF, WO = range(10)

GELU_C0 = 0.7978845608028654
GELU_C1 = 0.044715

BODY = (
    ('dwo0',),
    ('dma',),
    ('ds',),
    ('df',),
    ('dwf',),
    ('dwo1',),
    ('bp',),
    ('b64',),
    ('dhe',),
    ('dho',),
    ('n2',),
    ('w2',),
    ('dwo2',),
    ('ps',),
    ('dxc',),
    ('dxa',),
    ('dxb',),
    ('tr',),
    ('w1w',),
    ('as',),
    ('m2',),
    ('ho',),
    ('he',),
    ('hop',),
    ('es',),
    ('w1b',),
    ('hep',),
    ('nn',),
    ('t',),
    ('w1a',),
    ('w1c',),
    ('fp',),
    ('fe',),
    ('dwo3',),
    ('joint', 'dwo3'),
)


def _nn(a, w):
    return jnp.dot(a, w, preferred_element_type=f32)


def _nt(a, w):
    return lax.dot_general(a, w, (((1,), (1,)), ((), ())), preferred_element_type=f32)


def _tn(a, b):
    return lax.dot_general(a, b, (((0,), (0,)), ((), ())), preferred_element_type=f32)


def _gelu_parts(x):
    t = (GELU_C0 * GELU_C1) * (x * x)
    th = jnp.tanh(x * (GELU_C0 + t))
    s = 0.5 + 0.5 * th
    return t, th, s, x * s


def _gelu(x):
    return _gelu_parts(x)[3]


def _gelu_and_grad(x):
    t, th, s, g = _gelu_parts(x)
    return g, s + g * (1.0 - th) * (GELU_C0 + 3.0 * t)


def _cat(lo, hi):
    return jnp.concatenate([lo, hi], axis=1)


def _stack(a, b):
    return jnp.concatenate([a, b], axis=0)


def _halves(v):
    return v[:, :H], v[:, H:]


def _keep_rows(v, lo, hi):
    n = v.shape[0]
    a = -(-lo // 8) * 8
    b = hi // 8 * 8
    zero = jnp.zeros((), v.dtype)
    parts = []
    if a > 0:
        r = lax.broadcasted_iota(jnp.int32, (a, v.shape[1]), 0)
        parts.append(jnp.where(r >= lo, v[:a], zero))
    if b > a:
        parts.append(v[a:b])
    if b < n:
        r = lax.broadcasted_iota(jnp.int32, (n - b, v.shape[1]), 0) + b
        parts.append(jnp.where(r < hi, v[b:], zero))
    return jnp.concatenate(parts, axis=0) if len(parts) > 1 else parts[0]


def _zero_row_if(v, row, cond):
    if cond is False:
        return v
    a = row // 8 * 8
    blk = v[a:a + 8]
    r = lax.broadcasted_iota(jnp.int32, blk.shape, 0) + a
    kill = row if cond is True else jnp.where(cond, row, -1)
    blk = jnp.where(r == kill, jnp.zeros((), v.dtype), blk)
    parts = ([v[:a]] if a > 0 else []) + [blk] + ([v[a + 8:]] if a + 8 < v.shape[0] else [])
    return jnp.concatenate(parts, axis=0) if len(parts) > 1 else parts[0]


def _fwd_set(x11, x12, x21, x22):
    return [x11 + x22, x12 + x22, x11, x22, x11 + x21, x12 - x11, x21 - x22]


def _bwd_set(y11, y12, y21, y22):
    return [y11 + y22, y21 + y22, y11, y22, y11 + y12, y21 - y11, y12 - y22]


def _std_out(m):
    return m[0] + m[3] - m[4] + m[6], m[2] + m[4], m[1] + m[3], m[0] - m[1] + m[2] + m[5]


def _dual_out(n):
    return n[0] + n[3] - n[4] + n[6], n[1] + n[3], n[2] + n[4], n[0] - n[1] + n[2] + n[5]


def _zero_after(v):
    u = lax.bitcast_convert_type(v[:8, :H], u32)
    return lax.shift_right_logical(lax.shift_right_logical(u, jnp.uint32(31)), jnp.uint32(1))


def _products(fn, toks=None):
    m = [None] * 7
    for k in ORDER:
        m[k] = fn(k)
        if toks is not None:
            toks += [_zero_after(m[k]), _zero_after(m[k][m[k].shape[0] // 2:])]
    return m


def _tok(toks, i, n):
    return toks[i * len(toks) // n] if toks else None


def _after(vals, tok):
    if tok is None:
        return list(vals)
    out = []
    for v in vals:
        z = jnp.tile(tok, (v.shape[0] // 8, 1))
        out.append(v | z if v.dtype == u32 else v + lax.bitcast_convert_type(z, f32))
    return out


def _lo(w):
    return pltpu.unpack_elementwise(w, index=0, packed_dtype=bf16, unpacked_dtype=f32)


def _hi(w):
    return pltpu.unpack_elementwise(w, index=1, packed_dtype=bf16, unpacked_dtype=f32)


def _pack(a, b):
    return pltpu.pack_elementwise([a, b], packed_dtype=bf16)


def _words(v):
    return pltpu.bitcast(v, u32)


def _rows(w):
    return pltpu.bitcast(w, bf16)


def _aligned(v):
    return v if isinstance(v, int) else pl.multiple_of(v, 8)


def _kernel(x_hbm, go_hbm, g_hbm, w1_hbm, w2_hbm, wf_hbm, wg_hbm, wo_hbm,
            out_hbm, dx_hbm, dw1_hbm, dw2_hbm, dg_hbm, dwf_hbm, dwg_hbm, dwo_hbm,
            xbuf, gbuf, obuf, dxbuf,
            g_ref, w1_ref, w2_ref, wf_ref, wg_ref, wo_ref, wfs_ref, wtr_ref,
            as_ref, at_ref, m2_ref, hep_ref, hop_ref, fp_ref, hes_ref, het_ref, hof_ref, es_ref, ht_ref,
            fs_ref, ft_ref, ghe_ref, gho_ref, gf_ref, fe_ref, xs_ref, jt_ref, gs_ref, gu_ref,
            ds_ref, du_ref, dpf_ref, bs_ref, bu_ref, b64_ref, pm_ref, pef_ref, pof_ref, ps_ref,
            fold, ge_ref,
            acc1, acc2, acc2w, accf, acco, accg, dge_ref,
            dw1_st, dw2_st, dwf_st, dwo_st, dwg_st, dg_st,
            in_sem, out_sem, w_sem, dw_sem):

    def x_copy(step, h):
        nominal = step * (4 * TR) - 8
        if isinstance(step, int):
            src = min(max(nominal, 0), B * T - XD)
        else:
            src = jnp.clip(nominal, 0, B * T - XD)
        return pltpu.make_async_copy(
            x_hbm.at[pl.ds(_aligned(src), XD), pl.ds(h * H, H)],
            xbuf.at[step, h, pl.ds(_aligned(8 + src - nominal), XD), :],
            in_sem.at[step, h])

    def g_copy(step, h):
        return pltpu.make_async_copy(
            go_hbm.at[pl.ds(_aligned(step * (TR * U)), TR * U), pl.ds(h * H, H)],
            gbuf.at[step, h, pl.ds(U, TR * U), :],
            in_sem.at[step, 2 + h])

    def gh_copy(step, h):
        nominal = (step + 1) * (TR * U)
        if isinstance(step, int):
            src = min(nominal, B * R * U - U)
        else:
            src = jnp.minimum(nominal, B * R * U - U)
        return pltpu.make_async_copy(
            go_hbm.at[pl.ds(_aligned(src), U), pl.ds(h * H, H)],
            gbuf.at[step, h, pl.ds(U + TR * U, U), :],
            in_sem.at[step, 4 + h])

    def o_copy(step, h):
        return pltpu.make_async_copy(
            obuf.at[step, h, pl.ds(U, TR * U), :],
            out_hbm.at[pl.ds(_aligned(step * (TR * U)), TR * U), pl.ds(h * H, H)],
            out_sem.at[step, h])

    def dx_copy(step, h):
        return pltpu.make_async_copy(
            dxbuf.at[step, h, pl.ds(8, 4 * TR), :],
            dx_hbm.at[pl.ds(_aligned(step * (4 * TR)), 4 * TR), pl.ds(h * H, H)],
            out_sem.at[step, 2 + h])

    w_in = dict(w1=(w1_hbm, w1_ref), w2=(w2_hbm, w2_ref), wf=(wf_hbm, wf_ref),
                wo=(wo_hbm, wo_ref), g=(g_hbm, g_ref), wg=(wg_hbm, wg_ref))
    w_cp = {k: pltpu.make_async_copy(s, d, w_sem.at[i]) for i, (k, (s, d)) in enumerate(w_in.items())}

    def start(cp, step):
        for h in range(2):
            cp(step, h).start()

    def wait(cp, step):
        for h in range(2):
            cp(step, h).wait()

    fin = []

    def flush(src, dst):
        cp = pltpu.make_async_copy(src, dst, dw_sem.at[len(fin)])
        cp.start()
        fin.append(cp)

    def packed(v):
        return v.astype(bf16)

    def ld(ref, *idx, rows=None):
        view = ref.at[idx].bitcast(u32)
        return _rows(view[...] if rows is None else view[pl.ds(0, rows // 2), :])

    def snn(*pairs, toks=None):
        return _dual_out(_products(
            lambda k: functools.reduce(jnp.add, [_nn(lhs(PERM[k]), ld(wfs_ref, w, k)) for lhs, w in pairs]),
            toks))

    def snt(lhs, w, toks=None):
        return _std_out(_products(lambda k: _nt(lhs(k), ld(wfs_ref, w, PERM[k])), toks))

    def snt_pre(lhs, x, toks=None):
        return _std_out(_products(lambda k: _nn(lhs(k), _rows(wtr_ref[x, k])), toks))

    def stn(xt, y, toks=None):
        return _products(lambda k: _nn(xt(k), y(PERM[k])), toks)

    def join(c):
        return _stack(_cat(c[0], c[1]), _cat(c[2], c[3]))

    def with_halo(main, halo):
        return lambda k: _stack(ld(main, k, rows=H - CH_C), ld(halo, k))

    def chunk(ref, s):
        return [ref[q, pl.ds(s, CH_C), :] for q in range(4)]

    def eo_chunk(ref, s):
        return [ref[h, par, pl.ds(8 + s, CH_C), :] for par in range(2) for h in range(2)]

    def eo_quad(ref, par, delta, s):
        return [ref[h, par, pl.ds(8 + delta + s + r * (Q // 2), CH_C), :] for r in range(2) for h in range(2)]

    def eo_store(ref, blocks):
        for q, v in enumerate(blocks):
            ref[q % 2, q // 2, pl.ds(8, Q), :] = v

    def transpose_set(dst, src):
        for q in range(7):
            dst[q] = _words(ld(src, q).T)

    def accumulate(acc, prods, final):
        m = [acc[k] + functools.reduce(jnp.add, [p[k] for p in prods]) for k in range(7)]
        if final:
            return join(_std_out(m))
        for k in range(7):
            acc[k] = m[k]

    LAST = Q - CH_C
    HALO_ROW = TR // 2 - LAST
    J_PLAIN = ((2, 7), (8, 3))

    def without_halo(blocks):
        return blocks[:2] + [_zero_row_if(v, HALO_ROW, True) for v in blocks[2:]]

    def store_bwd_set(main, halo, blocks, s, halo_blocks=None):
        for q, v in enumerate(_bwd_set(*blocks)):
            main[q, pl.ds(s, CH_C), :] = packed(v)
        if halo_blocks is not None:
            for q, v in enumerate(_bwd_set(*halo_blocks)):
                halo[q] = packed(v)


    def st_as(step, first, toks):
        xw = [xbuf.at[step, h].bitcast(u32) for h in range(2)]
        for s in range(0, Q, CH_C):
            tok = _tok(toks, s, Q)

            def words(start):
                return _after([xw[h][pl.ds(start + 4 * s, CH_C, stride=4), :] for h in range(2)], tok)

            w01e, w23e = words(6), words(7)
            if s == 0:
                w01e = [_zero_row_if(w, 0, first) for w in w01e]
                w23e = [_zero_row_if(w, 0, first) for w in w23e]
            w01o, w23o, w23se = words(8), words(9), words(5)
            a1 = [_hi(w) for w in w01e + w01o]
            a3 = [_hi(w) for w in w23e + w23o]
            a3s = [_hi(w) for w in w23se] + a3[:2]
            ops = ([u - v for u, v in zip(a3s, a1)], a1, [u - v for u, v in zip(a3, a1)],
                   [_lo(w) for w in w01e + w01o], [_lo(w) for w in w23e + w23o])
            for k, blocks in enumerate(ops):
                for q, v in enumerate(_fwd_set(*blocks)):
                    as_ref[k, q, pl.ds(s, CH_C), :] = packed(v)

    def st_tr():
        for k in range(5):
            transpose_set(at_ref.at[k], as_ref.at[k])

    def a_op(k):
        return lambda q: ld(as_ref, k, q)

    def st_m2():
        toks = []
        for q, v in enumerate(snn((a_op(1), WS), toks=toks)):
            m2_ref[q] = v
        return toks

    def st_he():
        toks = []
        for q, v in enumerate(snn((a_op(3), W11), (a_op(0), W10), toks=toks)):
            hep_ref[q] = v + m2_ref[q]
        return toks

    def st_ho():
        toks = []
        for q, v in enumerate(snn((a_op(4), W11), (a_op(2), W12), toks=toks)):
            hop_ref[q] = v + m2_ref[q]
        return toks

    def activation(pre, grad_ref, s, tok):
        x = _after(chunk(pre, s), tok)
        if grad_ref is None:
            return [_gelu(v) for v in x]
        gs = [_gelu_and_grad(v) for v in x]
        for q in range(4):
            grad_ref[q, pl.ds(s, CH_C), :] = gs[q][1]
        return [g[0] for g in gs]

    def activation_set(pre, grad_ref, set_ref, t_ref, toks):
        for s in range(0, Q, CH_C):
            for q, v in enumerate(_fwd_set(*activation(pre, grad_ref, s, _tok(toks, s, Q)))):
                set_ref[q, pl.ds(s, CH_C), :] = packed(v)
        transpose_set(t_ref, set_ref)

    def st_grad(pre, grad_ref, toks):
        for s in range(0, Q, CH_C):
            activation(pre, grad_ref, s, _tok(toks, s, Q))

    def st_hep(toks, grad=True):
        activation_set(hep_ref, ghe_ref if grad else None, hes_ref, het_ref, toks)

    def st_hop(toks, grad=True):
        for s in range(0, Q, CH_C):
            for q, g in enumerate(activation(hop_ref, gho_ref if grad else None, s, _tok(toks, s, Q))):
                hof_ref[q % 2, q // 2, pl.ds(8 + s, CH_C), :] = g

    def st_es(toks):
        for s in range(0, Q // 2, CH_C):
            tok = _tok(toks, s, Q // 2)
            e, o, os_ = (_after(eo_quad(hof_ref, par, delta, s), tok) for par, delta in ((0, 0), (1, 0), (1, -1)))
            ops = ([u - v for u, v in zip(os_, e)], e, [u - v for u, v in zip(o, e)])
            for k, blocks in enumerate(ops):
                for q, v in enumerate(_fwd_set(*blocks) + [blocks[1], blocks[2]]):
                    es_ref[k, q, pl.ds(s, CH_C), :] = packed(v)
        for k in range(3):
            ht_ref[k] = _words(join([ld(es_ref, k, q) for q in (2, 7, 8, 3)]).T)

    def st_nn():
        toks = []
        n2 = snn((lambda q: ld(es_ref, 1, q), VS), toks=toks)
        n1 = snn((lambda q: ld(es_ref, 0, q), V0), toks=toks)
        n3 = snn((lambda q: ld(es_ref, 2, q), V2), toks=toks)
        for h in range(2):
            fp_ref[h] = _stack(n1[h] + n2[h], n1[2 + h] + n2[2 + h])
            fp_ref[2 + h] = _stack(n2[h] + n3[h], n2[2 + h] + n3[2 + h])
        return toks

    def st_t():
        toks = []
        for q, v in enumerate(snn((lambda q: ld(hes_ref, q), V1), toks=toks)):
            fp_ref[q] += v
        return toks

    def st_fp(toks, grad=True):
        activation_set(fp_ref, gf_ref if grad else None, fs_ref, ft_ref, toks)

    def st_fe():
        toks = []
        for q, v in enumerate(snn((lambda q: ld(fs_ref, q), WF), toks=toks)):
            fe_ref[q % 2, pl.ds(q // 2, Q, stride=2), :] = v
        return toks

    def st_j(step, p, toks):
        b = step // NT
        ge0 = [jnp.broadcast_to(ge_ref[h, pl.ds(b * U + 2 * p, 1), :], (CH_V, H)) for h in range(2)]
        ge1 = [jnp.broadcast_to(ge_ref[h, pl.ds(b * U + 2 * p + 1, 1), :], (CH_V, H)) for h in range(2)]
        for s in range(0, Q, CH_V):
            blk0, blk1 = [], []
            tok = _tok(toks, s, Q)
            g0, g1 = _after(ge0, tok), _after(ge1, tok)
            for r in range(2):
                for h in range(2):
                    fe = fe_ref[h, pl.ds(Q * r + s, CH_V), :]
                    blk0.append(jnp.tanh(fe + g0[h]))
                    blk1.append(jnp.tanh(fe + g1[h]))
            for q, (c0, c1) in enumerate(zip(_fwd_set(*blk0), _fwd_set(*blk1))):
                xs_ref[p, q, pl.ds(s, CH_V), :] = _pack(c0, c1)
            xs_ref[p, 7, pl.ds(s, CH_V), :] = _pack(blk0[1], blk1[1])
            xs_ref[p, 8, pl.ds(s, CH_V), :] = _pack(blk0[2], blk1[2])
        for q in range(7):
            jt_ref[p, q] = _words(_rows(xs_ref[p, q]).T)

    def g_plain(step, p, r, s, n):
        return gbuf.at[step, r].bitcast(u32)[pl.ds(p + 4 * (Q * r + s), n, stride=4), :]

    def st_g(step, p, toks):
        def operands(w11, w12, w21, w22):
            ws = (w11, w12, w21, w22)
            s0 = _bwd_set(*[_lo(w) for w in ws])
            s1 = _bwd_set(*[_hi(w) for w in ws])
            return [None if q in (2, 3) else _pack(c0, c1) for q, (c0, c1) in enumerate(zip(s0, s1))]

        for s in range(0, Q, CH_V):
            gw = _after([gbuf.at[step, h].bitcast(u32)[pl.ds(p + 4 * (Q * r + s), CH_V, stride=4), :]
                         for r in range(2) for h in range(2)], _tok(toks, s, Q))
            ops = operands(*gw)
            if s + CH_V == Q:
                for q in (0, 1, 4, 5, 6):
                    gu_ref[q] = ops[q]
                keep = TR + 1 - Q - s
                ops = operands(gw[0], gw[1], _keep_rows(gw[2], 0, keep), _keep_rows(gw[3], 0, keep))
            for q in (0, 1, 4, 5, 6):
                gs_ref[p, q if q < 2 else q - 2, pl.ds(s, CH_V), :] = ops[q]

    def st_dj(step, p):
        b = step // NT
        dge = [None, None]
        toks = []
        for s in range(0, Q, CH_DJ):
            def lhs(k):
                if k in (2, 3):
                    return g_plain(step, p, k - 2, s, CH_DJ)
                kk = k if k < 2 else k - 2
                if s + CH_DJ < Q:
                    return gs_ref[p, kk, pl.ds(s, CH_DJ), :]
                return _stack(gs_ref[p, kk, pl.ds(s, CH_DJ - 8), :], gu_ref[k])

            m = _products(lambda k: _nn(_rows(lhs(k)), _rows(wtr_ref[3, k])))
            c = _std_out(m)
            toks += [_zero_after(m[k][r:]) for k in (1, 0) for r in (0, CH_DJ)]
            for r in range(2):
                for n in range(2):
                    jf = _rows(xs_ref[p, J_PLAIN[r][n], pl.ds(s, CH_DJ), :]).astype(f32)
                    dz = c[2 * r + n] * (1.0 - jf * jf)
                    row0 = 2 * (Q * r + s)
                    if p == 0:
                        fold[n, pl.ds(row0, 2 * CH_DJ), :] = dz
                    else:
                        fold[n, pl.ds(row0, 2 * CH_DJ), :] += dz
                    hi = 2 * (TR + 1) - row0
                    if hi < 2 * CH_DJ:
                        dz = _keep_rows(dz, 0, hi)
                    part = jnp.sum(dz.reshape(2 * CH_DJ // 8, 8, H), axis=0)
                    dge[n] = part if dge[n] is None else dge[n] + part
        accg[b, p] += _cat(dge[0], dge[1])
        return toks

    def st_out(step, p):
        toks = []
        for s in range(0, Q, CH_OUT):
            n = _products(lambda k: _nn(_rows(xs_ref[p, PERM[k], pl.ds(s, CH_OUT), :]), ld(wfs_ref, WO, k)))
            c = _dual_out(n)
            toks += [_zero_after(n[k][r:]) for k in (1, 0) for r in (0, CH_OUT)]
            for r in range(2):
                for h in range(2):
                    ow = obuf.at[step, h].bitcast(u32)
                    ow[pl.ds(p + 4 * (Q * r + s), CH_OUT, stride=4), :] = _words(c[2 * r + h].astype(bf16))
        return toks

    def st_dwo(step, p, final=False):
        def rhs(q):
            if q not in (2, 3):
                return gs_ref[p, q if q < 2 else q - 2]
            w = g_plain(step, p, q - 2, 0, Q)
            return w if q == 2 else _keep_rows(w, 0, TR + 1 - Q)

        toks = []
        prod = _products(lambda k: _nn(_rows(jt_ref[p, k]), _rows(rhs(PERM[k]))), toks)
        r = accumulate(acco, [prod], final)
        if final:
            dwo_st[...] = r.astype(bf16)
            flush(dwo_st, dwo_hbm)
        return toks

    def joint_all(step, toks):
        st_g(step, 0, None)
        st_j(step, 0, toks)
        for p in range(4):
            t_dj = st_dj(step, p)
            if p < 3:
                st_g(step, p + 1, t_dj)
            t_out = st_out(step, p)
            if p < 3:
                st_j(step, p + 1, t_out)
        start(o_copy, step)

    def st_ds(last, toks):
        for s in range(0, Q, CH_C):
            tok = _tok(toks, s, Q)
            lo = _after([fold[h, pl.ds(2 * par + 4 * s, CH_C, stride=4), :]
                         for par in range(2) for h in range(2)], tok)
            blocks = [v + fold[q % 2, pl.ds(2 * (q // 2) + 1 + 4 * s, CH_C, stride=4), :] for q, v in enumerate(lo)]
            if s == LAST:
                halo = blocks[:2] + [_zero_row_if(v, HALO_ROW, last) for v in blocks[2:]]
                store_bwd_set(ds_ref, du_ref, without_halo(blocks), s, halo)
            else:
                store_bwd_set(ds_ref, du_ref, blocks, s)

    def st_df():
        toks = []
        df = snt(with_halo(ds_ref, du_ref), WF, toks)
        eo_store(dpf_ref, [v * gf_ref[q] for q, v in enumerate(df)])
        return toks

    def st_dwf(final=False):
        toks = []
        r = accumulate(accf, [stn(lambda k: _rows(ft_ref[k]), lambda q: ld(ds_ref, q), toks)], final)
        if final:
            dwf_st[...] = r.astype(bf16)
            flush(dwf_st, dwf_hbm)
        return toks

    def st_bp(toks):
        for s in range(0, Q, CH_C):
            blocks = _after(eo_chunk(dpf_ref, s), _tok(toks, s, Q))
            if s == LAST:
                masked = without_halo(blocks)
                store_bwd_set(bs_ref, bu_ref, masked, s, blocks)
            else:
                masked = blocks
                store_bwd_set(bs_ref, bu_ref, masked, s)
            for h in range(2):
                dem, dom = masked[h], masked[2 + h]
                for k, v in enumerate((dem, dem + dom, dom)):
                    pm_ref[k, h, pl.ds(s, CH_C), :] = packed(v)

    def st_b64(toks):
        for s in range(0, Q // 2, CH_C):
            tok = _tok(toks, s, Q // 2)
            de, do, des = (_after(eo_quad(dpf_ref, par, delta, s), tok) for par, delta in ((0, 0), (1, 0), (0, 1)))
            ops = (do, [u - v for u, v in zip(de, do)], [u - v for u, v in zip(des, do)])
            for k, blocks in enumerate(ops):
                for q, v in enumerate(_bwd_set(*blocks)):
                    b64_ref[k, q, pl.ds(s, CH_C), :] = packed(v)

    def st_dhe():
        toks = []
        dhe = snt(with_halo(bs_ref, bu_ref), V1, toks)
        eo_store(pef_ref, [v * ghe_ref[q] for q, v in enumerate(dhe)])
        return toks

    def st_dho():
        toks = []
        c = snt_pre(lambda q: ld(b64_ref, 0, q), 2, toks)
        x1 = snt_pre(lambda q: ld(b64_ref, 1, q), 1, toks)
        x2 = snt_pre(lambda q: ld(b64_ref, 2, q), 0, toks)
        for h in range(2):
            pof_ref[h] = _stack(x1[h] + c[h], x1[2 + h] + c[2 + h]) * gho_ref[h]
            pof_ref[2 + h] = _stack(c[h] + x2[h], c[2 + h] + x2[2 + h]) * gho_ref[2 + h]
        return toks

    def st_n2(final=False):
        n = [_nn(_rows(ht_ref[k]), _cat(ld(pm_ref, k, 0), ld(pm_ref, k, 1))) for k in (1, 0, 2)]
        n2, n1, n3 = (acc2[k] + v for k, v in zip((1, 0, 2), n))
        if final:
            dw2_st[0] = (n1 + n2).astype(bf16)
            dw2_st[2] = (n2 + n3).astype(bf16)
        else:
            acc2[0], acc2[1], acc2[2] = n1, n2, n3
        return [_zero_after(v[r:]) for v in n for r in (0, Q // 2, Q, 3 * Q // 2)]

    def st_w2(final=False):
        toks = []
        r = accumulate(acc2w, [stn(lambda k: _rows(het_ref[k]), lambda q: ld(bs_ref, q), toks)], final)
        if final:
            dw2_st[1] = r.astype(bf16)
        return toks

    def st_ps(toks):
        for s in range(0, Q, CH_C):
            tok = _tok(toks, s, Q)
            pe = _after(eo_chunk(pef_ref, s), tok)
            pes = pe[2:] + _after([pef_ref[h, 0, pl.ds(8 + s + 1, CH_C), :] for h in range(2)], tok)
            po = _after(chunk(pof_ref, s), tok)
            if s == 0:
                po = [_zero_row_if(v, 0, True) for v in po[:2]] + po[2:]
            if s == LAST:
                pe, po = without_halo(pe), without_halo(po)
            sl = pl.ds(s, CH_C)
            for q, (e, o, es) in enumerate(zip(_bwd_set(*pe), _bwd_set(*po), _bwd_set(*pes))):
                ps_ref[0, q, sl, :] = packed(e)
                ps_ref[1, q, sl, :] = packed(o)
                ps_ref[2, q, sl, :] = packed(e - o)
                ps_ref[3, q, sl, :] = packed(es - o)
                ps_ref[4, q, sl, :] = packed(e + o)

    def pset(k):
        return lambda q: ld(ps_ref, k, q)

    def st_dxc():
        toks = []
        for q, v in enumerate(snt(pset(1), WS, toks)):
            m2_ref[q] = v
        return toks

    def dx_half(step, first, plain, outer, offset):
        toks = []
        da = snt(pset(plain), W11, toks)
        db = snt(pset(outer[0]), outer[1], toks)
        for q in range(4):
            dxw = dxbuf.at[step, q % 2].bitcast(u32)
            dxw[pl.ds(offset + 2 * (q // 2), Q, stride=4), :] = _pack(da[q], db[q] + m2_ref[q])
        return toks

    def st_dxa(step):
        return dx_half(step, True, 0, (2, W12), 2)

    def st_dxb(step):
        toks = dx_half(step, False, 1, (3, W10), 3)
        start(dx_copy, step)
        return toks

    def st_w1(k, final=False):
        toks = []
        pairs = {3: [(3, 0), (4, 1)], 1: [(1, 4)], 0: [(0, 0)], 2: [(2, 1)]}[k]
        prods = [stn(lambda q, n=n: _rows(at_ref[n, q]), pset(y), toks) for n, y in pairs]
        r = accumulate(acc1.at[k], prods, final)
        return r if final else toks

    zb = jnp.zeros

    def clear_margins(s):
        for h in range(2):
            xbuf[s, h, pl.ds(0, 16), :] = zb((16, H), bf16)
            xbuf[s, h, pl.ds(XD, XW - XD), :] = zb((XW - XD, H), bf16)
            gbuf[s, h, pl.ds(0, U), :] = zb((U, H), bf16)
            gbuf[s, h, pl.ds(GD, GW - GD), :] = zb((GW - GD, H), bf16)

    def zero_blocks(ref, n):
        def blk(k, carry):
            ref[k] = zb(ref.shape[1:], ref.dtype)
            return carry
        lax.fori_loop(0, n, blk, 0)

    def clear_rest(k, carry):
        clear_margins(k)
        return carry

    def weight_blocks(w):
        w = w.astype(f32)
        return [w[:H, :H], w[:H, H:], w[H:, :H], w[H:, H:]]

    def weight_set(idx, blocks, tr=None):
        ops = [packed(v) for v in _fwd_set(*blocks)]
        for k in range(7):
            wfs_ref[idx, k] = ops[k]
            if tr is not None:
                wtr_ref[tr, k] = _words(ops[PERM[k]].T)

    def tap_sets(w_ref, first, tr):
        b0, b1, b2 = (weight_blocks(w_ref[k]) for k in range(3))
        weight_set(first + 3, [u + v for u, v in zip(b0, b2)], tr[2])
        weight_set(first + 1, b1)
        weight_set(first, b0, tr[0])
        weight_set(first + 2, b2, tr[1])

    clear_margins(0)
    start(x_copy, 0)
    zero_blocks(acc1, 4)
    w_cp["w1"].start()
    zero_blocks(acc2, 3)
    w_cp["w2"].start()
    zero_blocks(accg, B)
    w_cp["wf"].start()
    zero_blocks(hof_ref, 2)
    for k in ("g", "wg", "wo"):
        w_cp[k].start()
    zero_blocks(dpf_ref, 2)
    start(g_copy, 0)
    start(gh_copy, 0)
    lax.fori_loop(1, NSTEP, clear_rest, 0)
    start(x_copy, 1)
    zero_blocks(pef_ref, 2)
    start(g_copy, 1)
    start(gh_copy, 1)
    for ref in (accf, acco, acc2w):
        ref[...] = zb(ref.shape, f32)
    wait(x_copy, 0)
    st_as(0, True, None)
    w_cp["w1"].wait()
    tap_sets(w1_ref, W10, (None, None, None))
    st_m2()
    st_ho()
    t_he = st_he()
    st_hop(None)
    st_es(None)
    st_hep(None)
    for k in ("w2", "wf", "g", "wg", "wo"):
        w_cp[k].wait()
    tap_sets(w2_ref, V0, (0, 1, 2))
    weight_set(WF, weight_blocks(wf_ref[...]))
    weight_set(WO, weight_blocks(wo_ref[...]), 3)
    ge = _nn(g_ref[...], wg_ref[...])
    for h, vh in enumerate(_halves(ge)):
        ge_ref[h] = vh
    st_nn()
    st_t()
    st_fp(None)
    st_fe()
    t_out = None
    for p in range(4):
        st_j(0, p, t_out)
        t_out = st_out(0, p)
    wait(g_copy, 0)
    wait(gh_copy, 0)
    st_g(0, 0, None)
    for p in range(4):
        t_dj = st_dj(0, p)
        if p < 3:
            st_g(0, p + 1, t_dj)

    def body(i, carry):
        wait(x_copy, i + 1)
        wait(g_copy, i + 1)
        wait(gh_copy, i + 1)
        last = i % NT == NT - 1
        first = (i + 1) % NT == 0
        toks = {}

        def dma():
            @pl.when(i == 0)
            def _():
                start(o_copy, 0)

            @pl.when(i + 2 < NSTEP)
            def _():
                start(x_copy, i + 2)
                start(g_copy, i + 2)
                start(gh_copy, i + 2)

        stages = dict(
            dma=lambda t: dma(),
            dwo0=lambda t: st_dwo(i, 0), dwo1=lambda t: st_dwo(i, 1),
            dwo2=lambda t: st_dwo(i, 2), dwo3=lambda t: st_dwo(i, 3),
            ds=lambda t: st_ds(last, t), df=lambda t: st_df(), dwf=lambda t: st_dwf(),
            bp=st_bp, b64=st_b64, dhe=lambda t: st_dhe(), dho=lambda t: st_dho(),
            n2=lambda t: st_n2(), w2=lambda t: st_w2(), ps=st_ps,
            dxc=lambda t: st_dxc(), dxa=lambda t: st_dxa(i), dxb=lambda t: st_dxb(i),
            tr=lambda t: st_tr(),
            w1w=lambda t: st_w1(3), w1b=lambda t: st_w1(1), w1a=lambda t: st_w1(0), w1c=lambda t: st_w1(2),
            **{"as": lambda t: st_as(i + 1, first, t)},
            m2=lambda t: st_m2(), he=lambda t: st_he(), ho=lambda t: st_ho(),
            hep=st_hep, hop=st_hop, es=st_es,
            hep0=lambda t: st_hep(t, False), hop0=lambda t: st_hop(t, False), fp0=lambda t: st_fp(t, False),
            ghe=lambda t: st_grad(hep_ref, ghe_ref, t), gho=lambda t: st_grad(hop_ref, gho_ref, t),
            gf=lambda t: st_grad(fp_ref, gf_ref, t),
            nn=lambda t: st_nn(), t=lambda t: st_t(), fp=st_fp, fe=lambda t: st_fe(),
            joint=lambda t: joint_all(i + 1, t),
        )
        for name, *sources in BODY:
            toks[name] = stages[name]([z for src in sources for z in toks[src]] or None)
        return carry

    lax.fori_loop(0, NSTEP - 1, body, 0)

    last = NSTEP - 1
    st_dwo(last, 0)
    st_ds(True, None)
    st_df()
    t = st_dwf(final=True)
    t = t + st_dwo(last, 1)
    st_bp(t)
    st_b64(None)
    for b in range(B):
        for p in range(4):
            a = accg[b, p]
            a = a + pltpu.roll(a, 6, 0)
            a = a + pltpu.roll(a, 4, 0)
            dge_ref[pl.ds(b * U + 2 * p, 2), :] = a[0:2]
    dge = dge_ref[...].astype(bf16)
    dg_st[...] = _nt(dge, wg_ref[...]).astype(bf16)
    dwg_st[...] = _tn(g_ref[...], dge).astype(bf16)
    flush(dg_st, dg_hbm)
    flush(dwg_st, dwg_hbm)
    st_dhe()
    st_dho()
    t = st_n2(final=True) + st_w2(final=True)
    flush(dw2_st, dw2_hbm)
    t = t + st_dwo(last, 2)
    st_ps(t)
    st_dwo(last, 3, final=True)
    st_dxc()
    st_dxa(last)
    st_dxb(last)
    st_tr()
    dw1_st[1] = st_w1(3, True).astype(bf16)
    flush(dw1_st.at[1], dw1_hbm.at[1])
    m2 = st_w1(1, True)
    dw1_st[0] = (st_w1(0, True) + m2).astype(bf16)
    flush(dw1_st.at[0], dw1_hbm.at[0])
    dw1_st[2] = (m2 + st_w1(2, True)).astype(bf16)
    flush(dw1_st.at[2], dw1_hbm.at[2])
    for step in range(NSTEP):
        wait(o_copy, step)
        wait(dx_copy, step)
    for cp in fin:
        cp.wait()


@jax.jit
def pallas_standalone__seq2seq_rnn_t_joint__speech_kernel(x, w1, w2, g, w_f, w_g, w_o, grad_out):
    x2 = x.reshape(B * T, D)
    go2 = grad_out.reshape(B * R * U, D)
    g2 = g.reshape(B * U, D)
    hbm = pl.BlockSpec(memory_space=pl.ANY)
    sds = jax.ShapeDtypeStruct
    vmem = pltpu.VMEM
    out, dx, dw1, dw2, dg, dwf, dwg, dwo = pl.pallas_call(
        _kernel,
        in_specs=[hbm] * 8,
        out_specs=[hbm] * 8,
        out_shape=[sds((B * R * U, D), bf16), sds((B * T, D), bf16), sds((3, D, D), bf16),
                   sds((3, D, D), bf16), sds((B * U, D), bf16), sds((D, D), bf16),
                   sds((D, D), bf16), sds((D, D), bf16)],
        scratch_shapes=[
            vmem((NSTEP, 2, XW, H), bf16),
            vmem((NSTEP, 2, GW, H), bf16),
            vmem((NSTEP, 2, GW, H), bf16),
            vmem((NSTEP, 2, DXW, H), bf16),
            vmem((B * U, D), bf16),
            vmem((3, D, D), bf16),
            vmem((3, D, D), bf16),
            vmem((D, D), bf16),
            vmem((D, D), bf16),
            vmem((D, D), bf16),
            vmem((10, 7, H, H), bf16),
            vmem((4, 7, HW, H), u32),
            vmem((5, 7, H, H), bf16),
            vmem((5, 7, HW, H), u32),
            vmem((4, H, H), f32),
            vmem((4, H, H), f32),
            vmem((4, H, H), f32),
            vmem((4, H, H), f32),
            vmem((7, H, H), bf16),
            vmem((7, HW, H), u32),
            vmem((2, 2, Q + 16, H), f32),
            vmem((3, 9, HW, H), bf16),
            vmem((3, D // 2, Q), u32),
            vmem((7, H, H), bf16),
            vmem((7, HW, H), u32),
            vmem((4, H, H), f32),
            vmem((4, H, H), f32),
            vmem((4, H, H), f32),
            vmem((2, M + 8, H), f32),
            vmem((4, 9, Q, H), u32),
            vmem((4, 7, H // 2, M), u32),
            vmem((4, 5, Q, H), u32),
            vmem((7, 8, H), u32),
            vmem((7, H, H), bf16),
            vmem((7, CH_C, H), bf16),
            vmem((2, 2, Q + 16, H), f32),
            vmem((7, H, H), bf16),
            vmem((7, CH_C, H), bf16),
            vmem((3, 7, HW, H), bf16),
            vmem((3, 2, Q, H), bf16),
            vmem((2, 2, Q + 16, H), f32),
            vmem((4, H, H), f32),
            vmem((5, 7, H, H), bf16),
            vmem((2, 2 * M + 8, H), f32),
            vmem((2, B * U, H), f32),
            vmem((4, 7, H, H), f32),
            vmem((3, D, D), f32),
            vmem((7, H, H), f32),
            vmem((7, H, H), f32),
            vmem((7, H, H), f32),
            vmem((B, 4, 8, D), f32),
            vmem((B * U, D), f32),
            vmem((3, D, D), bf16),
            vmem((3, D, D), bf16),
            vmem((D, D), bf16),
            vmem((D, D), bf16),
            vmem((D, D), bf16),
            vmem((B * U, D), bf16),
            pltpu.SemaphoreType.DMA((NSTEP, 6)),
            pltpu.SemaphoreType.DMA((NSTEP, 4)),
            pltpu.SemaphoreType.DMA((6,)),
            pltpu.SemaphoreType.DMA((8,)),
        ],
        compiler_params=pltpu.CompilerParams(vmem_limit_bytes=100 * 1024 * 1024,
                                             disable_bounds_checks=True,
                                             disable_semaphore_checks=True),
    )(x2, go2, g2, w1, w2, w_f, w_g, w_o)
    return (out.reshape(B, R, U, D), dx.reshape(B, T, D), dw1, dw2, dg.reshape(B, U, D),
            dwf, dwg, dwo)
```
